```python
import os as _os
_os.environ.setdefault("JAX_PLATFORMS", "cpu")
import jax
import jax.numpy as jnp

def _softmax(x, axis=-1):
    return jax.nn.softmax(x, axis=axis)
def _gelu(x):
    return jax.nn.gelu(x, approximate=True)
def _silu(x):
    return jax.nn.silu(x)
def _sigmoid(x):
    return jax.nn.sigmoid(x)
def _layernorm(x, axis=-1, eps=1e-5):
    m = jnp.mean(x, axis=axis, keepdims=True)
    v = jnp.var(x, axis=axis, keepdims=True)
    return (x - m) / jnp.sqrt(v + eps)
def _scatter_add(tgt, idx, src, axis=0):
    return tgt.at[idx].add(src)
def _segment_sum(src, seg, n):
    return jax.ops.segment_sum(src, seg, n)
class _Rng:
    def __init__(self, key):
        self._k = key
    def _next(self):
        self._k, sub = jax.random.split(self._k)
        return sub
    def normal(self, shape):
        return jax.random.normal(self._next(), shape, dtype=jnp.bfloat16)
    def randint(self, lo, hi, shape):
        return jax.random.randint(self._next(), shape, lo, hi, dtype=jnp.int32)
    def uniform(self, shape, lo=0.0, hi=1.0):
        return jax.random.uniform(self._next(), shape, jnp.bfloat16, lo, hi)
    def permutation(self, n):
        return jax.random.permutation(self._next(), n)


kernel_name = 'concat_heads__gqa_block_cached__gqa_block_cached__near_ridge'

def setup_inputs():
    _rng = _Rng(jax.random.key(int.from_bytes(__import__("os").urandom(4), "little")))
    _w = (lambda a: (lambda t: t.astype(jnp.bfloat16) if jnp.issubdtype(t.dtype, jnp.floating) else t)(jnp.asarray(a)))
    def _A_setup():
        B, Sq, D = 8, 240, 640
        Hq, Hkv, Sk, Dh = 32, 32, 1024, 192
        assert Hq % Hkv == 0, (Hq, Hkv)
        return {
            "x": _w((lambda *s: _rng.normal(s) * 0.8)(B, Sq, D)),
            "k_cache": _w((lambda *s: _rng.normal(s) * 0.8)(B, Hkv, Sk, Dh)),
            "v_cache": _w((lambda *s: _rng.normal(s) * 0.05)(B, Hkv, Sk, Dh)),
            "wq": _w((lambda *s: _rng.normal(s) * 0.8)(D, Hq * Dh) * (D ** -0.5)),
            "wo": _w((lambda *s: _rng.normal(s) * 0.05)(Hq * Dh, D) * ((Hq * Dh) ** -0.5)),
        }
    _A_in = _A_setup()

    def _B_setup():
        B, Sq, D = 8, 240, 640
        Hq, Hkv, Sk, Dh = 32, 32, 1024, 192
        assert Hq % Hkv == 0, (Hq, Hkv)
        return {
            "x": _w((lambda *s: _rng.normal(s) * 0.8)(B, Sq, D)),
            "k_cache": _w((lambda *s: _rng.normal(s) * 0.8)(B, Hkv, Sk, Dh)),
            "v_cache": _w((lambda *s: _rng.normal(s) * 0.05)(B, Hkv, Sk, Dh)),
            "wq": _w((lambda *s: _rng.normal(s) * 0.8)(D, Hq * Dh) * (D ** -0.5)),
            "wo": _w((lambda *s: _rng.normal(s) * 0.05)(Hq * Dh, D) * ((Hq * Dh) ** -0.5)),
        }
    _B_in = _B_setup()

    return {
        "A_x": _A_in["x"],
        "A_k_cache": _A_in["k_cache"],
        "A_v_cache": _A_in["v_cache"],
        "A_wq": _A_in["wq"],
        "A_wo": _A_in["wo"],
        "B_x": _B_in["x"],
        "B_k_cache": _B_in["k_cache"],
        "B_v_cache": _B_in["v_cache"],
        "B_wq": _B_in["wq"],
        "B_wo": _B_in["wo"],
    }

def reference(A_x, A_k_cache, A_v_cache, A_wq, A_wo, B_x, B_k_cache, B_v_cache, B_wq, B_wo):
    def _A_ref(x, k_cache, v_cache, wq, wo):
        B, Sq, D = x.shape
        Hq, Dh = 32, 192
        Hkv = k_cache.shape[1]
        rep = Hq // Hkv
        q = (lambda x, *d: x.transpose(*d))((x @ wq).reshape(B, Sq, Hq, Dh), 0, 2, 1, 3)
        k = jnp.repeat(k_cache, rep, axis=1)
        v = jnp.repeat(v_cache, rep, axis=1)
        scores = jnp.einsum("bhqd,bhkd->bhqk", q, k) * (Dh ** -0.5)
        p = _softmax(scores, axis=-1)
        o = jnp.einsum("bhqk,bhkd->bhqd", p, v)
        return (lambda x, *d: x.transpose(*d))(o, 0, 2, 1, 3).reshape(B, Sq, Hq * Dh) @ wo

    def _B_ref(x, k_cache, v_cache, wq, wo):
        B, Sq, D = x.shape
        Hq, Dh = 32, 192
        Hkv = k_cache.shape[1]
        rep = Hq // Hkv
        q = (lambda x, *d: x.transpose(*d))((x @ wq).reshape(B, Sq, Hq, Dh), 0, 2, 1, 3)
        k = jnp.repeat(k_cache, rep, axis=1)
        v = jnp.repeat(v_cache, rep, axis=1)
        scores = jnp.einsum("bhqd,bhkd->bhqk", q, k) * (Dh ** -0.5)
        p = _softmax(scores, axis=-1)
        o = jnp.einsum("bhqk,bhkd->bhqd", p, v)
        return (lambda x, *d: x.transpose(*d))(o, 0, 2, 1, 3).reshape(B, Sq, Hq * Dh) @ wo

    a = _A_ref(A_x, A_k_cache, A_v_cache, A_wq, A_wo)
    b = _B_ref(B_x, B_k_cache, B_v_cache, B_wq, B_wo)
    return jnp.concatenate([a, b], axis=-1)
```

```python
import functools

import jax
import jax.numpy as jnp
import jax.experimental.pallas as pl
import jax.experimental.pallas.tpu as pltpu


def _attn_pair(x, k_ref, v_ref, wq, wo, *, hp, dh):
    scale = dh ** -0.5
    q_all = jnp.dot(x, wq, preferred_element_type=jnp.float32) * scale
    outs = []
    for j in range(hp):
        q = q_all[:, j * dh:(j + 1) * dh].astype(jnp.bfloat16)
        k = k_ref[0, j]
        v = v_ref[0, j]
        s = jax.lax.dot_general(q, k, (((1,), (1,)), ((), ())),
                                preferred_element_type=jnp.float32)
        m = jnp.max(s, axis=-1, keepdims=True)
        p = jnp.exp(s - m)
        l = jnp.sum(p, axis=-1, keepdims=True)
        o = jnp.dot(p.astype(jnp.bfloat16), v, preferred_element_type=jnp.float32)
        outs.append((o / l).astype(jnp.bfloat16))
    o_all = jnp.concatenate(outs, axis=-1) if hp > 1 else outs[0]
    return jnp.dot(o_all, wo, preferred_element_type=jnp.float32)


def _kernel(ax_ref, ak_ref, av_ref, awq_ref, awo_ref,
            bx_ref, bk_ref, bv_ref, bwq_ref, bwo_ref,
            o_ref, acc_ref, *, hp, dh, d):
    h = pl.program_id(1)

    @pl.when(h == 0)
    def _():
        acc_ref[...] = jnp.zeros_like(acc_ref)

    acc_ref[:, 0:d] += _attn_pair(ax_ref[0], ak_ref, av_ref, awq_ref[...], awo_ref[...], hp=hp, dh=dh)
    acc_ref[:, d:2 * d] += _attn_pair(bx_ref[0], bk_ref, bv_ref, bwq_ref[...], bwo_ref[...], hp=hp, dh=dh)

    @pl.when(h == pl.num_programs(1) - 1)
    def _():
        o_ref[0] = acc_ref[...].astype(o_ref.dtype)


@jax.jit
def pallas_concat_heads__gqa_block_cached__gqa_block_cached__near_ridge_kernel(
    A_x: jax.Array,
    A_k_cache: jax.Array,
    A_v_cache: jax.Array,
    A_wq: jax.Array,
    A_wo: jax.Array,
    B_x: jax.Array,
    B_k_cache: jax.Array,
    B_v_cache: jax.Array,
    B_wq: jax.Array,
    B_wo: jax.Array,
):
    B, Sq, D = A_x.shape
    _, Hkv, Sk, Dh = A_k_cache.shape
    Hq = A_wq.shape[1] // Dh
    assert Hq == Hkv
    HP = 2

    x_spec = pl.BlockSpec((1, Sq, D), lambda b, h: (b, 0, 0))
    kv_spec = pl.BlockSpec((1, HP, Sk, Dh), lambda b, h: (b, h, 0, 0))
    wq_spec = pl.BlockSpec((D, HP * Dh), lambda b, h: (0, h))
    wo_spec = pl.BlockSpec((HP * Dh, D), lambda b, h: (h, 0))
    one = [x_spec, kv_spec, kv_spec, wq_spec, wo_spec]

    return pl.pallas_call(
        functools.partial(_kernel, hp=HP, dh=Dh, d=D),
        grid=(B, Hq // HP),
        in_specs=one + one,
        out_specs=pl.BlockSpec((1, Sq, 2 * D), lambda b, h: (b, 0, 0)),
        out_shape=jax.ShapeDtypeStruct((B, Sq, 2 * D), A_x.dtype),
        scratch_shapes=[pltpu.VMEM((Sq, 2 * D), jnp.float32)],
        compiler_params=pltpu.CompilerParams(
            dimension_semantics=("parallel", "arbitrary"),
            vmem_limit_bytes=100 * 1024 * 1024,
        ),
    )(A_x, A_k_cache, A_v_cache, A_wq, A_wo, B_x, B_k_cache, B_v_cache, B_wq, B_wo)
```

```python
import functools

import jax
import jax.numpy as jnp
import jax.experimental.pallas as pl
import jax.experimental.pallas.tpu as pltpu

_NT = (((1,), (1,)), ((), ()))


def _attn_pair(x, kt_ref, vt_ref, wq, wo, *, hp, dh):
    scale = dh ** -0.5
    q_all = (jnp.dot(x, wq, preferred_element_type=jnp.float32) * scale).astype(jnp.bfloat16)
    ots, rs = [], []
    for j in range(hp):
        q = q_all[:, j * dh:(j + 1) * dh]
        s = jnp.dot(q, kt_ref[0, j], preferred_element_type=jnp.float32)
        m = jnp.max(s, axis=-1, keepdims=True)
        p = jnp.exp(s - m)
        l = jnp.sum(p, axis=-1, keepdims=True)
        ot = jax.lax.dot_general(vt_ref[0, j], p.astype(jnp.bfloat16), _NT,
                                 preferred_element_type=jnp.float32)
        ots.append(ot)
        rs.append(1.0 / l)
    o_all = jnp.concatenate(ots, axis=0).T
    lane = jax.lax.broadcasted_iota(jnp.int32, o_all.shape, 1)
    r = rs[-1]
    for j in range(hp - 2, -1, -1):
        r = jnp.where(lane < (j + 1) * dh, rs[j], r)
    o_all = (o_all * r).astype(jnp.bfloat16)
    return jnp.dot(o_all, wo, preferred_element_type=jnp.float32)


def _kernel(ax_ref, ak_ref, av_ref, awq_ref, awo_ref,
            bx_ref, bk_ref, bv_ref, bwq_ref, bwo_ref,
            o_ref, acc_ref, *, hp, dh, d):
    h = pl.program_id(1)

    @pl.when(h == 0)
    def _():
        acc_ref[...] = jnp.zeros_like(acc_ref)

    acc_ref[:, 0:d] += _attn_pair(ax_ref[0], ak_ref, av_ref, awq_ref[...], awo_ref[...], hp=hp, dh=dh)
    acc_ref[:, d:2 * d] += _attn_pair(bx_ref[0], bk_ref, bv_ref, bwq_ref[...], bwo_ref[...], hp=hp, dh=dh)

    @pl.when(h == pl.num_programs(1) - 1)
    def _():
        o_ref[0] = acc_ref[...].astype(o_ref.dtype)


@jax.jit
def pallas_concat_heads__gqa_block_cached__gqa_block_cached__near_ridge_kernel(
    A_x: jax.Array,
    A_k_cache: jax.Array,
    A_v_cache: jax.Array,
    A_wq: jax.Array,
    A_wo: jax.Array,
    B_x: jax.Array,
    B_k_cache: jax.Array,
    B_v_cache: jax.Array,
    B_wq: jax.Array,
    B_wo: jax.Array,
):
    B, Sq, D = A_x.shape
    _, Hkv, Sk, Dh = A_k_cache.shape
    Hq = A_wq.shape[1] // Dh
    assert Hq == Hkv
    HP = 2

    tr = lambda a: jnp.swapaxes(a, 2, 3)

    x_spec = pl.BlockSpec((1, Sq, D), lambda b, h: (b, 0, 0))
    kv_spec = pl.BlockSpec((1, HP, Dh, Sk), lambda b, h: (b, h, 0, 0))
    wq_spec = pl.BlockSpec((D, HP * Dh), lambda b, h: (0, h))
    wo_spec = pl.BlockSpec((HP * Dh, D), lambda b, h: (h, 0))
    one = [x_spec, kv_spec, kv_spec, wq_spec, wo_spec]

    return pl.pallas_call(
        functools.partial(_kernel, hp=HP, dh=Dh, d=D),
        grid=(B, Hq // HP),
        in_specs=one + one,
        out_specs=pl.BlockSpec((1, Sq, 2 * D), lambda b, h: (b, 0, 0)),
        out_shape=jax.ShapeDtypeStruct((B, Sq, 2 * D), A_x.dtype),
        scratch_shapes=[pltpu.VMEM((Sq, 2 * D), jnp.float32)],
        compiler_params=pltpu.CompilerParams(
            dimension_semantics=("parallel", "arbitrary"),
            vmem_limit_bytes=100 * 1024 * 1024,
        ),
    )(A_x, tr(A_k_cache), tr(A_v_cache), A_wq, A_wo, B_x, tr(B_k_cache), tr(B_v_cache), B_wq, B_wo)
```

```python
import functools

import jax
import jax.numpy as jnp
import jax.experimental.pallas as pl
import jax.experimental.pallas.tpu as pltpu

_NT = (((1,), (1,)), ((), ()))
_LOG2E = 1.4426950408889634
CK = 512


def _kernel(ax_ref, ak_ref, av_ref, awq_ref, awo_ref,
            bx_ref, bk_ref, bv_ref, bwq_ref, bwo_ref,
            o_ref, acc_ref, *, hp, dh, d, sk):
    h = pl.program_id(1)

    @pl.when(h == 0)
    def _():
        acc_ref[...] = jnp.zeros_like(acc_ref)

    scale = dh ** -0.5 * _LOG2E
    nc = sk // CK
    qa = (jnp.dot(ax_ref[0], awq_ref[...], preferred_element_type=jnp.float32) * scale).astype(jnp.bfloat16)
    qb = (jnp.dot(bx_ref[0], bwq_ref[...], preferred_element_type=jnp.float32) * scale).astype(jnp.bfloat16)
    units = [(qa, ak_ref, av_ref, j) for j in range(hp)] + [(qb, bk_ref, bv_ref, j) for j in range(hp)]

    def qk_chunk(u, c):
        qq, k_ref, _, j = units[u]
        return jnp.dot(qq[:, j * dh:(j + 1) * dh], k_ref[0, j, :, c * CK:(c + 1) * CK],
                       preferred_element_type=jnp.float32)

    s_next = [qk_chunk(0, c) for c in range(nc)]
    ots, rs = [], []
    for u in range(len(units)):
        s = s_next
        s_next = []
        mx = s[0]
        for c in range(1, nc):
            mx = jnp.maximum(mx, s[c])
        m = jnp.max(mx, axis=-1, keepdims=True)
        v_ref, j = units[u][2], units[u][3]
        ot = None
        ls = None
        for c in range(nc):
            p = jnp.exp2(s[c] - m)
            ls = p if ls is None else ls + p
            o_c = jax.lax.dot_general(v_ref[0, j, :, c * CK:(c + 1) * CK], p.astype(jnp.bfloat16), _NT,
                                      preferred_element_type=jnp.float32)
            ot = o_c if ot is None else ot + o_c
            if u + 1 < len(units):
                s_next.append(qk_chunk(u + 1, c))
        ots.append(ot)
        rs.append(1.0 / jnp.sum(ls, axis=-1, keepdims=True))

    for prob, wo_ref in enumerate((awo_ref, bwo_ref)):
        o_all = jnp.concatenate(ots[prob * hp:(prob + 1) * hp], axis=0).T
        lane = jax.lax.broadcasted_iota(jnp.int32, o_all.shape, 1)
        rr = rs[prob * hp:(prob + 1) * hp]
        r = rr[-1]
        for j in range(hp - 2, -1, -1):
            r = jnp.where(lane < (j + 1) * dh, rr[j], r)
        o_all = (o_all * r).astype(jnp.bfloat16)
        acc_ref[:, prob * d:(prob + 1) * d] += jnp.dot(o_all, wo_ref[...], preferred_element_type=jnp.float32)

    @pl.when(h == pl.num_programs(1) - 1)
    def _():
        o_ref[0] = acc_ref[...].astype(o_ref.dtype)


@jax.jit
def pallas_concat_heads__gqa_block_cached__gqa_block_cached__near_ridge_kernel(
    A_x, A_k_cache, A_v_cache, A_wq, A_wo, B_x, B_k_cache, B_v_cache, B_wq, B_wo,
):
    B, Sq, D = A_x.shape
    _, Hkv, Sk, Dh = A_k_cache.shape
    Hq = A_wq.shape[1] // Dh
    assert Hq == Hkv
    HP = 4

    tr = lambda a: jnp.swapaxes(a, 2, 3)

    x_spec = pl.BlockSpec((1, Sq, D), lambda b, h: (b, 0, 0))
    kv_spec = pl.BlockSpec((1, HP, Dh, Sk), lambda b, h: (b, h, 0, 0))
    wq_spec = pl.BlockSpec((D, HP * Dh), lambda b, h: (0, h))
    wo_spec = pl.BlockSpec((HP * Dh, D), lambda b, h: (h, 0))
    one = [x_spec, kv_spec, kv_spec, wq_spec, wo_spec]

    return pl.pallas_call(
        functools.partial(_kernel, hp=HP, dh=Dh, d=D, sk=Sk),
        grid=(B, Hq // HP),
        in_specs=one + one,
        out_specs=pl.BlockSpec((1, Sq, 2 * D), lambda b, h: (b, 0, 0)),
        out_shape=jax.ShapeDtypeStruct((B, Sq, 2 * D), A_x.dtype),
        scratch_shapes=[pltpu.VMEM((Sq, 2 * D), jnp.float32)],
        compiler_params=pltpu.CompilerParams(
            dimension_semantics=("parallel", "arbitrary"),
            vmem_limit_bytes=100 * 1024 * 1024,
        ),
    )(A_x, tr(A_k_cache), tr(A_v_cache), A_wq, A_wo, B_x, tr(B_k_cache), tr(B_v_cache), B_wq, B_wo)
```
